```python
import jax
import jax.numpy as jnp

def _softmax(x, axis=-1):
    return jax.nn.softmax(x, axis=axis)
def _gelu(x):
    return jax.nn.gelu(x, approximate=True)
def _silu(x):
    return jax.nn.silu(x)
def _sigmoid(x):
    return jax.nn.sigmoid(x)
def _layernorm(x, axis=-1, eps=1e-5):
    m = jnp.mean(x, axis=axis, keepdims=True)
    v = jnp.var(x, axis=axis, keepdims=True)
    return (x - m) / jnp.sqrt(v + eps)
def _scatter_add(tgt, idx, src, axis=0):
    return tgt.at[idx].add(src)
def _segment_sum(src, seg, n):
    return jax.ops.segment_sum(src, seg, n)
class _Rng:
    def __init__(self, key):
        self._k = key
    def _next(self):
        self._k, sub = jax.random.split(self._k)
        return sub
    def normal(self, shape):
        return jax.random.normal(self._next(), shape, dtype=jnp.bfloat16)
    def randint(self, lo, hi, shape):
        return jax.random.randint(self._next(), shape, lo, hi, dtype=jnp.int32)
    def uniform(self, shape, lo=0.0, hi=1.0):
        return jax.random.uniform(self._next(), shape, jnp.bfloat16, lo, hi)
    def permutation(self, n):
        return jax.random.permutation(self._next(), n)


kernel_name = 'parallel_sum__sliding_local_dilated__mixer_channel_mlp__prompt'

def _fwd_setup_inputs():
    _rng = _Rng(jax.random.key(int.from_bytes(__import__("os").urandom(4), "little")))
    _w = (lambda a: (lambda t: t.astype(jnp.bfloat16) if jnp.issubdtype(t.dtype, jnp.floating) else t)(jnp.asarray(a)))
    def _A_setup():
        B, S, D = 1, 2048, 576
        return {
            "x": _w((lambda *s: _rng.normal(s) * 0.05)(B, S, D)),
            "wqkv": _w((lambda *s: _rng.normal(s) * 0.05)(D, 3 * D)),
            "wo": _w((lambda *s: _rng.normal(s) * 0.05)(D, D)),
        }
    _A_in = _A_setup()

    def _B_setup():
        B, S, D, F = 1, 2048, 576, 4608
        return {
            "x": _w((lambda *s: _rng.normal(s) * 0.05)(B, S, D)),
            "w1": _w((lambda *s: _rng.normal(s) * 0.05)(D, F) * (D ** -0.5)),
            "b1": _w((lambda *s: _rng.normal(s) * 0.05)(F)),
            "w2": _w((lambda *s: _rng.normal(s) * 0.05)(F, D) * (F ** -0.5)),
            "b2": _w((lambda *s: _rng.normal(s) * 0.05)(D)),
        }
    _B_in = _B_setup()

    return {
        "A_x": _A_in["x"],
        "A_wqkv": _A_in["wqkv"],
        "A_wo": _A_in["wo"],
        "B_x": _B_in["x"],
        "B_w1": _B_in["w1"],
        "B_b1": _B_in["b1"],
        "B_w2": _B_in["w2"],
        "B_b2": _B_in["b2"],
    }

def _fwd_reference(A_x, A_wqkv, A_wo, B_x, B_w1, B_b1, B_w2, B_b2):
    def _A_ref(x, wqkv, wo):
        B, S, D = x.shape
        H = 32; Dh = D // H
        W, dil = 8, 2
        qkv = (lambda x, *d: x.transpose(*d))((x @ wqkv).reshape(B, S, 3, H, Dh), 2, 0, 3, 1, 4)
        q, k, v = qkv[0], qkv[1], qkv[2]
        scale = Dh ** -0.5
        pos = jnp.arange(S)
        off = jnp.arange(W) * dil
        idx = pos[:, None] - off[None, :]
        mask = idx >= 0
        idx_c = jnp.where(mask, idx, 0).reshape(-1)
        kg = k[:, :, idx_c, :].reshape(B, H, S, W, Dh)
        vg = v[:, :, idx_c, :].reshape(B, H, S, W, Dh)
        logits = jnp.einsum("bhsd,bhswd->bhsw", q, kg) * scale
        logits = jnp.where(mask[None, None, :, :], logits, -1e9)
        attn = _softmax(logits, axis=-1)
        o = jnp.einsum("bhsw,bhswd->bhsd", attn, vg)
        return (lambda x, *d: x.transpose(*d))(o, 0, 2, 1, 3).reshape(B, S, D) @ wo

    def _B_ref(x, w1, b1, w2, b2):
        y = _layernorm(x, axis=-1)
        h = _gelu(jnp.einsum("bsd,df->bsf", y, w1) + b1)
        return jnp.einsum("bsf,fd->bsd", h, w2) + b2

    x = A_x
    xn = _layernorm(x, axis=-1)
    return x + _A_ref(xn, A_wqkv, A_wo) + _B_ref(xn, B_w1, B_b1, B_w2, B_b2)


def setup_inputs():
    _inp = _fwd_setup_inputs()
    _gk = jax.random.fold_in(jax.random.key(int.from_bytes(__import__("os").urandom(4), "little")), 2**31 - 1)
    _shapes = [[1, 2048, 576]]
    _dtypes = ['bfloat16']
    _gks = jax.random.split(_gk, len(_shapes))
    _gs = [jax.random.normal(k, s, dtype=jnp.dtype(d)) * 0.05 for k, s, d in zip(_gks, _shapes, _dtypes)]
    _inp["grad_out"] = _gs[0]
    return _inp

def reference(A_x, A_wqkv, A_wo, B_w1, B_b1, B_w2, B_b2, B_x, grad_out):
    _const = dict(B_x=B_x)
    def _f(*_d):
        return _fwd_reference(**{'A_x': _d[0], 'A_wqkv': _d[1], 'A_wo': _d[2], 'B_w1': _d[3], 'B_b1': _d[4], 'B_w2': _d[5], 'B_b2': _d[6], **_const})
    _out, _vjp = jax.vjp(_f, A_x, A_wqkv, A_wo, B_w1, B_b1, B_w2, B_b2)
    _grads = _vjp(grad_out)
    _out0 = jnp.asarray(_out)
    return (_out0, *[jnp.asarray(_g) for _g in _grads])
```

```python
import jax
import jax.numpy as jnp
from jax import lax
import jax.experimental.pallas as pl
import jax.experimental.pallas.tpu as pltpu

S, D, F = 2048, 576, 4608
H, DH, W, DIL = 32, 18, 8, 2
EPS = 1e-5
FC = 512
NCH = F // FC
CG = 512
NG = S // CG
NB = S // 128
DP = D // 2
HP = DH // 2
HG = 8
HF, HD, HS = FC // 2, D // 2, S // 2
NIT = 2 * NCH
HQ = 3 * HD
KQ = 896
KS = (256, 256, 384, 384, 256, 384, 384)
BF, F32, U32 = jnp.bfloat16, jnp.float32, jnp.uint32
C1 = 0.7978845608028654
C2 = C1 * 0.044715


NN = (((1,), (0,)), ((), ()))
NT = (((1,), (1,)), ((), ()))


def _dot(a, b, dn):
    return lax.dot_general(a, b, dn, preferred_element_type=F32)


def _f(v):
    return v.astype(F32)


def _words(v):
    return pltpu.bitcast(v.astype(BF), U32)


def _bf(t):
    return pltpu.bitcast(t, BF)


def _unpack(t):
    return pltpu.bitcast(t << 16, F32), pltpu.bitcast(t & jnp.uint32(0xFFFF0000), F32)


def _pack(lo, hi):
    if 1:
        return pltpu.pack_elementwise([lo, hi], packed_dtype=BF)
    lo_b = pltpu.bitcast(lo.astype(BF).astype(F32), U32) >> 16
    hi_b = pltpu.bitcast(hi.astype(BF).astype(F32), U32)
    return lo_b | hi_b


def _ln_stats(v):
    m = jnp.sum(v, axis=0, keepdims=True) * (1.0 / D)
    c = v - m
    r = lax.rsqrt(jnp.sum(c * c, axis=0, keepdims=True) * (1.0 / D) + EPS)
    return c * r, m, r


def _ln_bwd(dy, y, r):
    m1 = jnp.sum(dy, axis=0, keepdims=True) * (1.0 / D)
    m2 = jnp.sum(dy * y, axis=0, keepdims=True) * (1.0 / D)
    return r * (dy - m1 - y * m2)


def _alpha(a11, a12, a21, a22):
    return [a11 + a22, a21 + a22, a11, a22, a11 + a12, a21 - a11, a12 - a22]


def _beta(b11, b12, b21, b22):
    return [b11 + b22, b11, b12 - b22, b21 - b11, b22, b11 + b12, b21 + b22]


def _gamma(c11, c12, c21, c22):
    return [c11 + c22, c21 - c22, c12 + c22, c11 + c21, c12 - c11, c22, c11]


def _combine(m):
    return m[0] + m[3] - m[4] + m[6], m[2] + m[4], m[1] + m[3], m[0] - m[1] + m[2] + m[5]


def _combine_t(n):
    return n[0] + n[2] + n[4] - n[5], n[4] + n[6], n[1] + n[5], n[0] + n[1] + n[3] - n[6]


def _rows(*u):
    return jnp.concatenate(u, axis=0)


def _beta_k(w, rem):
    n = w.shape[1] // 2
    b = _beta(w[0:256, :n], w[0:256, n:], w[256:512, :n], w[256:512, n:])
    r1, r2 = rem[:, :n], rem[:, n:]
    return [b[0], b[1], _rows(b[2], r2), _rows(b[3], r1), b[4], _rows(b[5], r2), _rows(b[6], r1)]


def _alpha_k(ta, tb, pad):
    a = _alpha(ta[0:256], ta[256:512], tb[0:256], tb[256:512])
    ra, rb = ta[512:D], tb[512:D]
    zero = jnp.zeros_like(pad)
    return [a[0], a[1], _rows(a[2], ra, pad), _rows(a[3], rb, pad), a[4],
            _rows(a[5], rb - ra, zero), _rows(a[6], ra - rb, zero)]


def _beta_kr(ta, tb, pad):
    b = _beta(ta[0:256], tb[0:256], ta[256:512], tb[256:512])
    r1, r2 = _rows(ta[512:D], pad), _rows(tb[512:D], pad)
    return [b[0], b[1], _rows(b[2], r2), _rows(b[3], r1), b[4], _rows(b[5], r2), _rows(b[6], r1)]


def _cols(*u):
    return jnp.concatenate(u, axis=1)


def _lazy(form, *parts):
    class Term:
        def __init__(self, get):
            self.get = get

        def __add__(self, other):
            return Term(lambda: self.get() + other.get())

        def __sub__(self, other):
            return Term(lambda: self.get() - other.get())
    return [t.get for t in form(*[Term(p) for p in parts])]


def _alpha_k_tiles(ga, gb, pad):
    out = []
    for t in range(2):
        r = t * 128
        forms = _lazy(_alpha, lambda r=r: ga(r, 128), lambda r=r: ga(256 + r, 128),
                      lambda r=r: gb(r, 128), lambda r=r: gb(256 + r, 128))
        out += [(k, t, v) for k, v in enumerate(forms)]
    zero = jnp.zeros_like(pad)
    out += [(2, 2, lambda: _rows(ga(512, 64), pad)), (3, 2, lambda: _rows(gb(512, 64), pad)),
            (5, 2, lambda: _rows(gb(512, 64) - ga(512, 64), zero)), (6, 2, lambda: _rows(ga(512, 64) - gb(512, 64), zero))]
    return out


def _tile(v, n):
    return _rows(*[v] * (n // 8))


def _fold(v):
    return jnp.sum(v.reshape(v.shape[0] // 8, 8, v.shape[1]), axis=0)


def _mean(part):
    return jnp.sum(part, axis=0, keepdims=True) * (1.0 / D)


def _gelu(pre, dh, c2):
    x2c = (c2 * pre) * pre
    ht = 0.5 * jnp.tanh(pre * (C1 + x2c))
    sg = 0.5 + ht
    h = pre * sg
    return h, dh * (sg + h * (0.5 - ht) * (2.0 * C1 + 6.0 * x2c))


def _interleave(main, n_main, *side):
    done = [0] * len(side)
    for k in range(n_main):
        for q, (gen, n) in enumerate(side):
            while done[q] < (k * n) // (n_main - 1):
                next(gen)
                done[q] += 1
        next(main)
    for gen in (main, *[g for g, _ in side]):
        assert next(gen, None) is None


def _chain(*gens):
    for g in gens:
        yield from g


def _take(gen, n):
    for _ in range(n):
        yield next(gen)


def _run(gen):
    for _ in gen:
        pass


class _Order:
    def __init__(self, zero):
        self.zero = zero
        self.pending = []
        self.last = None

    def note(self, *vs):
        vs = [v if v.dtype == U32 else pltpu.bitcast(v, U32) for v in vs]
        vs = [v[:, c:c + 128] for v in vs for c in range(0, v.shape[1], 128)]
        out = vs[0]
        for v in vs[1:]:
            out = out | v
        self.pending.append(out)

    def note_all(self, v, rows):
        for r in range(0, v.shape[0], rows):
            self.note(*[v[rr:rr + 8, c:c + 128] for rr in range(r, min(r + rows, v.shape[0]), 8)
                        for c in range(0, v.shape[1], 128)])

    def dot(self, a, b, dn):
        ax = 1 if dn == NN else 0
        width = 128 if a.shape[1] >= 512 else 256
        blocks = [(c, min(c + width, b.shape[ax])) for c in range(0, b.shape[ax], width)]
        if not 1:
            blocks = [(0, b.shape[ax])]
        slots = [(u, kc, r) for u in range(len(blocks)) for kc in range(0, a.shape[1] - 127, 512)
                 for r in range(0, a.shape[0], 8)]
        at = {}
        for q, v in enumerate(self.pending):
            key = slots[q * len(slots) // len(self.pending)]
            at[key] = v if key not in at else at[key] | v
        self.pending = []
        out = []
        for u, (c0, c1) in enumerate(blocks):
            parts, prev = [], 0
            for r in sorted({r for (uu, _, r) in at if uu == u}):
                if r > prev:
                    parts.append(a[prev:r])
                row, pc = [], 0
                for kc in range(0, a.shape[1] - 127, 512):
                    if (u, kc, r) in at:
                        if kc > pc:
                            row.append(a[r:r + 8, pc:kc])
                        row.append(a[r:r + 8, kc:kc + 128] | (at[u, kc, r] & self.zero))
                        pc = kc + 128
                if pc < a.shape[1]:
                    row.append(a[r:r + 8, pc:])
                parts.append(_cols(*row))
                prev = r + 8
            if prev < a.shape[0]:
                parts.append(a[prev:])
            out.append(_dot(_bf(_rows(*parts)), b[:, c0:c1] if ax else b[c0:c1], dn))
        self.last, self.calls = (_rows(*[v[:, 0:128] for v in out]) if 0 else out[-1]), 0
        return _cols(*out)

    def hold(self, t, after=None):
        if after is None:
            if self.last is None:
                return t
            step = 48 if self.last.shape[0] == CG else 48
            r = min(self.calls * step, self.last.shape[0] - 8)
            self.calls += 1
            after = self.last[r:r + 8, 0:128]
        return t | (pltpu.bitcast(after, U32) & self.zero)

    def gate(self, v):
        v = pltpu.bitcast(jnp.broadcast_to(v, (8, v.shape[1])), U32)
        if self.last is not None and 1:
            u = pltpu.bitcast(self.last[0:8, 0:128], U32) & self.zero
            v = v | _cols(*[u] * (v.shape[1] // 128))
        return pltpu.bitcast(v, F32)


def _kernel(xT_hbm, gT_hbm, wqkv_hbm, wo_hbm, w1_hbm, b1_ref, w2T_hbm, b2_ref,
            outT_hbm, dxT_hbm, dwqkv_hbm, dwo_hbm, dw1_hbm, db1_ref, dw2T_hbm, db2_ref,
            xT, gT, wqkv, wo, tg, tx, oT, dqkvT, acc, hf, qT, doT, p_s, ds_s, db1s, ln_s, zero_s, dw_s,
            sem_x, sem_g, sem_w, sem_wc, sem_d, sem_o, sem_dx, sem_dw):

    def x_cp(j):
        return pltpu.make_async_copy(xT_hbm.at[:, pl.ds(j * CG, CG)], xT.at[j], sem_x.at[j])

    def g_cp(j):
        return pltpu.make_async_copy(gT_hbm.at[:, pl.ds(j * CG, CG)], gT.at[j], sem_g.at[j])

    def chunk(i):
        return pl.ds(i * FC if isinstance(i, int) else pl.multiple_of(i * FC, FC), FC)

    def d_cp(i, q):
        return pltpu.make_async_copy(dw_s.at[q], (dw1_hbm, dw2T_hbm)[q].at[:, chunk(i)], sem_d.at[q])

    wo_cp = [pltpu.make_async_copy(wo_hbm.at[r:r + 144], wo.at[r:r + 144], sem_w.at[r // 144]) for r in range(0, D, 144)]
    wqkv_cp = pltpu.make_async_copy(wqkv_hbm, wqkv, sem_w.at[4])
    rowp = lax.broadcasted_iota(jnp.int32, (64, 128), 0)
    ones_pad = jnp.where(rowp == 0, 1.0, 0.0)
    zero_pad = jnp.zeros((64, 128), F32)

    def clear(i, carry):
        zero_s[i] = jnp.zeros((8, 128), U32)
        return carry + i
    z = lax.fori_loop(0, 2, clear, -1)

    def fence():
        lax.fori_loop(1, z + 2, clear, 0)

    def _fine(main, n_main, *side, end=True):
        _interleave(main, n_main, *side)
        if end or not 1:
            fence()

    def zz(j):
        return z if isinstance(j, int) else 0

    scale = DH ** -0.5
    lane = lax.broadcasted_iota(jnp.int32, (HG, 128), 1)

    def back(prev, cur, w):
        if w == 0:
            return cur
        return pltpu.roll(jnp.where(lane >= 128 - DIL * w, prev, cur), DIL * w, 1)

    def fwd(cur, nxt, w):
        if w == 0:
            return cur
        return pltpu.roll(jnp.where(lane < DIL * w, nxt, cur), 128 - DIL * w, 1)

    def attn_stage2(c, hg, od):
        hs = pl.ds(hg * HG, HG)
        c = c + zz(c)
        for src, wt, off in ((qT, ds_s, DP), (doT, p_s, 2 * DP)):
            ws = [fwd(wt[c % 4, w, hs, :], wt[(c + 1) % 4, w, hs, :], w) for w in range(W)]
            for d in range(HP):
                rows = pl.ds(hg * HG * HP + d, HG, stride=HP)
                sc, sn = src[c, rows, :], src[c + 1, rows, :]
                sc = od.hold(sc)
                al = ah = None
                for w in range(W):
                    sl, sh = _unpack(fwd(sc, sn, w))
                    al = ws[w] * sl if w == 0 else al + ws[w] * sl
                    ah = ws[w] * sh if w == 0 else ah + ws[w] * sh
                res = _pack(al, ah)
                dst = pl.ds(off + hg * HG * HP + d, HG, stride=HP)
                dqkvT[c, dst, :] = res
                od.note(res)
                yield 1

    N1, N2 = 3 * HP + 1, 2 * HP

    def stage_e(i, q, out, od):
        for k in range(7):
            out.append(od.dot(tg[q, k], _bf(_rows(hf[i % 2, 0, q, k], hf[i % 2, 1, q, k])), NN))
            yield 1

    def finish_e(q, n, od):
        for r in range(0, HD, 48):
            for v, (r0, c0) in zip(_combine_t([u[r:r + 48] for u in n]), ((0, 0), (0, HF), (HD, 0), (HD, HF))):
                v = v.astype(BF)
                dw_s[q, r0 + r:r0 + r + 48, c0:c0 + HF] = v
                od.note_all(pltpu.bitcast(v, U32), 24)
            yield 1

    def main_phase(wc, b1s, ta0, ta1, kT, vT, hx, bf, af):
        ta = (ta0, ta1)

        def w_cps(i):
            return [pltpu.make_async_copy(src.at[:, chunk(i)], wc.at[i % 2, q], sem_wc.at[2 * (i % 2) + q])
                    for q, src in enumerate((w1_hbm, w2T_hbm))]

        def attn_stage1(c, hg, od):
            def rows(d):
                return pl.ds(hg * HG * HP + d, HG, stride=HP)
            hs = pl.ds(hg * HG, HG)
            lg = [None] * W
            c = c + zz(c)
            for d in range(HP):
                ql, qh = _unpack(qT[c, rows(d), :])
                kp, kc = kT[c, rows(d), :], kT[c + 1, rows(d), :]
                kc = od.hold(kc)
                for w in range(W):
                    kl, kh = _unpack(back(kp, kc, w))
                    t = ql * kl + qh * kh
                    lg[w] = t if d == 0 else lg[w] + t
                od.note(*lg)
                yield 1
            tok = lane + c * 128
            lg = [lg[0] * scale] + [jnp.where(tok >= DIL * w, lg[w] * scale, -1e9) for w in range(1, W)]
            m = lg[0]
            for w in range(1, W):
                m = jnp.maximum(m, lg[w])
            e = [jnp.exp(l - m) for l in lg]
            tot = e[0]
            for w in range(1, W):
                tot = tot + e[w]
            inv = 1.0 / tot
            p = [x * inv for x in e]
            od.note(inv)
            yield 1
            dp = [None] * W
            for d in range(HP):
                gl, gh = _unpack(doT[c, rows(d), :])
                vp, vc = vT[c, rows(d), :], vT[c + 1, rows(d), :]
                vc = od.hold(vc)
                ol = oh = None
                for w in range(W):
                    vl, vh = _unpack(back(vp, vc, w))
                    t = gl * vl + gh * vh
                    dp[w] = t if d == 0 else dp[w] + t
                    ol = p[w] * vl if w == 0 else ol + p[w] * vl
                    oh = p[w] * vh if w == 0 else oh + p[w] * vh
                res = _pack(ol, oh)
                oT[c, rows(d), :] = res
                od.note(res, *dp)
                yield 1
            dot = p[0] * dp[0]
            for w in range(1, W):
                dot = dot + p[w] * dp[w]
            ds = [p[w] * (dp[w] - dot) * scale for w in range(W)]
            od.note(dot)
            for w in range(W):
                p_s[c % 4, w, hs, :] = p[w]
                ds_s[c % 4, w, hs, :] = ds[w]
            for d in range(HP):
                kp, kc = kT[c, rows(d), :], kT[c + 1, rows(d), :]
                kc = od.hold(kc)
                al = ah = None
                for w in range(W):
                    kl, kh = _unpack(back(kp, kc, w))
                    al = ds[w] * kl if w == 0 else al + ds[w] * kl
                    ah = ds[w] * kh if w == 0 else ah + ds[w] * kh
                res = _pack(al, ah)
                dqkvT[c, rows(d), :] = res
                od.note(res)
                yield 1

        row64 = lax.broadcasted_iota(jnp.int32, (64, FC), 0)

        def put(dst, forms, od):
            for k, v in enumerate(forms):
                v = _words(v)
                dst[k, 0:v.shape[0]] = v
                od.note_all(v, 32)
                yield 1

        def prep_b(i, q, od):
            wv = _f(wc[i % 2, q])
            brow = jnp.where(jnp.logical_and(row64 == 0, q == 0), jnp.broadcast_to(b1s[i][0:1], (64, FC)), 0.0)
            yield from put(bf.at[i % 2, q], _beta_k(wv, _rows(wv[512:D], brow)), od)

        def prep_a(i, q, od):
            wv = _f(wc[i % 2, q])
            yield from put(af.at[i % 2, q], _alpha(wv[0:HD, :HF], wv[0:HD, HF:], wv[HD:D, :HF], wv[HD:D, HF:]), od)

        def stage_a(i, j, qs, out, od):
            for q in qs:
                for k in range(7):
                    out.append(od.dot(ta[q][j + zz(j), k, :, 0:KS[k]], _bf(bf[i % 2 + zz(j), q, k, 0:KS[k] // 2]), NN))
                    yield 1

        GU = (CG // 16) * (HF // 128)

        def stage_g(i, j, m, od, after):
            sums = {}
            for u in range(GU):
                r, c = ((u // 2) * 16, (u % 2) * 128) if not 0 else ((u % 32) * 16, (u // 32) * 128)
                pre = _combine([v[r:r + 16, c:c + 128] for v in m[0:7]])
                dh = _combine([v[r:r + 16, c:c + 128] for v in m[7:14]])
                c2 = pltpu.bitcast(jnp.full((8, 128), C2, F32), U32)
                c2 = pltpu.bitcast(od.hold(c2, None if after is None else after(u)), F32)
                c2 = _rows(c2, c2)
                hd = [_gelu(p_, q_, c2) for p_, q_ in zip(pre, dh)]
                done = []
                for q in range(2):
                    h11, h12, h21, h22 = [v[1 - q] for v in hd]
                    for k, v in enumerate(_beta(h11, h21, h12, h22)):
                        v = _words(v)
                        hx[q, k, r // 2:r // 2 + 8, c:c + 128] = v
                        if k not in (1, 4) or not 0:
                            done.append(v)
                od.note(*done)
                for col, v in ((c, hd[0][1] + hd[2][1]), (HF + c, hd[1][1] + hd[3][1])):
                    v = v[0:8] + v[8:16]
                    sums[col] = v if col not in sums else sums[col] + v
                if u == GU - 1:
                    for col, v in sums.items():
                        db1s[i, j, :, col:col + 128] = v
                yield 1

        def stage_c(i, j, first, od):
            for q in (1, 0):
                for k in range(7):
                    v = hx[q + z, k]
                    hf[i % 2, j, q, k] = v
                    r = od.dot(af[i % 2 + zz(j), q, k], _bf(v), NT)
                    acc[q, j, k] = r if first else acc[q, j, k] + r
                    yield 1

        def init():
            zero_blk = jnp.zeros((DP, 128), U32)
            kT[0] = zero_blk
            vT[0] = zero_blk
            qT[NB] = zero_blk
            doT[NB] = zero_blk
            for blk in (NB - 1, NB):
                p_s[blk % 4] = jnp.zeros((W, H, 128), F32)
                ds_s[blk % 4] = jnp.zeros((W, H, 128), F32)
            b1f32 = _f(b1_ref[...]).reshape(1, F)
            for i in range(NCH):
                b1s[i] = jnp.broadcast_to(b1f32[:, i * FC:(i + 1) * FC], (8, FC))

        def prologue(rx0, rx1, bq, lnb, wqT):
            rx = (rx0, rx1)

            def tok_forms(j, c, ga, gb, pad, nat, raw, od):
                for k, t, get in _alpha_k_tiles(ga, gb, pad):
                    v = get().astype(BF)
                    if raw is not None:
                        u = pltpu.bitcast(v, U32)
                        raw[k, t * 64:(t + 1) * 64, c * 128:(c + 1) * 128] = u
                    if nat is not None:
                        u = pltpu.bitcast(v.T, U32)
                        nat[j, k, c * 64:(c + 1) * 64, t * 128:(t + 1) * 128] = u
                    od.note_all(u, 64)
                    yield 1

            def g_forms(j, od):
                for c in range(4):
                    ls = slice(c * 128, (c + 1) * 128)
                    yield from tok_forms(j, c, lambda r, n: _f(gT[j, r:r + n, ls]), lambda r, n: _f(gT[j + 2, r:r + n, ls]),
                                         zero_pad, ta[1], None, od)

            def grad_forms(j, get, od):
                for r in range(0, HD, 16):
                    for c in range(0, CG, 256):
                        ls = slice(c, c + 256)
                        for blocks in zip(get(j, r, ls), get(j + 2, r, ls), get(j, HD + r, ls), get(j + 2, HD + r, ls)):
                            done = [_words(v) for v in _gamma(*[v for _, v in blocks])]
                            for k, v in enumerate(done):
                                blocks[0][0][k, r // 2:r // 2 + 8, j * CG + c:j * CG + c + 256] = v
                            od.note(*done)
                        yield 1

            def g_rows(jj, r, ls):
                return [(tg.at[1], _f(gT[jj, r:r + 16, ls]))]

            def x_rows(jj, r, ls):
                m1, r1, m2, r2 = [ln_s[jj + z, e, 0:1, ls] for e in range(4)]
                xn = (_f(xT[jj, r:r + 16, ls]) - m1) * r1
                return [(tx, xn), (tg.at[0], (xn - m2) * r2)]

            def x_forms(j, od):
                for c in range(2):
                    ls = slice(c * 256, (c + 1) * 256)

                    def sweep(term):
                        tot = None
                        for r in range(0, D, 96):
                            v = [_fold(term(u, r)) for u in range(2)]
                            tot = v if tot is None else [tot[u] + v[u] for u in range(2)]
                            od.note(*tot)
                            yield 1
                        return [_mean(v) for v in tot]

                    def x(u, r):
                        return _f(xT[j + 2 * u, r:r + 96, ls])

                    def xn_new(u, r):
                        v = (x(u, r) - m1[u]) * r1[u]
                        lnb[0, u, r:r + 96] = v
                        return v

                    def xn(u, r):
                        return lnb[z, u, r:r + 96]
                    m1 = yield from sweep(x)
                    r1 = [lax.rsqrt(v + EPS) for v in (yield from sweep(lambda u, r: jnp.square(x(u, r) - m1[u])))]
                    m2 = yield from sweep(xn_new)
                    r2 = [lax.rsqrt(v + EPS) for v in (yield from sweep(lambda u, r: jnp.square(xn(u, r) - m2[u])))]
                    for u in range(2):
                        for e, v in enumerate((m1, r1, m2, r2)):
                            ln_s[j + 2 * u, e, :, ls] = jnp.broadcast_to(v[u], (8, 256))
                    for b in range(2):
                        bs = slice(b * 128, (b + 1) * 128)
                        xa, xb = [lambda r, n, u=u: lnb[z, u, r:r + n, bs] for u in range(2)]
                        ya, yb = [lambda r, n, u=u: (lnb[z, u, r:r + n, bs] - m2[u][:, bs]) * r2[u][:, bs] for u in range(2)]
                        yield from tok_forms(j, 2 * c + b, ya, yb, ones_pad, ta[0], None, od)
                        yield from tok_forms(j, 2 * c + b, xa, xb, zero_pad, None, rx[j], od)

            def wqkv_t(od):
                for c in range(0, 3 * D, 128):
                    n = min(128, 3 * D - c)
                    v = _rows(wqkv[:, c:c + n], jnp.zeros((64, n), BF)).T
                    wqT[c // 2:(c + n) // 2] = u = pltpu.bitcast(v, U32)
                    od.note_all(u, 64)
                    yield 1

            def w_forms(dst, w, n, od):
                for r in range(0, n, 48):
                    u, l = _f(w(r)), _f(w(n + r))
                    b = _beta(u[:, 0:256], l[:, 0:256], u[:, 256:512], l[:, 256:512])
                    r1, r2 = u[:, 512:640], l[:, 512:640]
                    forms = [b[0], b[1], _cols(b[2], r2), _cols(b[3], r1), b[4], _cols(b[5], r2), _cols(b[6], r1)]
                    for k, v in enumerate(forms):
                        v = _words(v)
                        dst[k, r // 2:r // 2 + 24, 0:KS[k]] = v
                        od.note_all(v, 24)
                    yield 1

            def proj(wf, src, m, od):
                for k in range(7):
                    m.append(od.dot(wf[k + z, :, 0:KS[k]], _bf(src[k + z, 0:KS[k] // 2]), NN))
                    yield 1

            def finish_proj(j, m, place, od):
                n = m[0].shape[0]
                for r in range(0, n, 48):
                    q = _combine([v[r:r + 48] for v in m])
                    for jj, r0, v in ((j, r, q[0]), (j, n + r, q[1]), (j + 2, r, q[2]), (j + 2, n + r, q[3])):
                        v = _words(v)
                        ref, shift, row = place(r0 // 2)
                        for b in range(4):
                            ref[jj * 4 + b + shift, row:row + 24] = v[:, b * 128:(b + 1) * 128]
                        od.note_all(v, 24)
                    yield 1

            def qkv_place(r):
                return ((qT, 0), (kT, 1), (vT, 1))[r // DP] + (r % DP,)

            def do_plain(j, od):
                for r in range(0, D, 144):
                    if j == 0:
                        wo_cp[r // 144].wait()
                    v = _words(od.dot(pltpu.bitcast(wo[r:r + 144], U32), gT[j], NN))
                    for b in range(4):
                        doT[j * 4 + b, r // 2:r // 2 + 72] = v[:, b * 128:(b + 1) * 128]
                    yield 1

            def stage(wait, start):
                for cp in wait:
                    cp.wait()
                for cp in start:
                    cp.start()

            w10, w20 = w_cps(0)
            stage((), (g_cp(0), *wo_cp))
            init()
            stage((g_cp(0),), (g_cp(2), w20))
            od = _Order(zero_s[0])
            mg0, mg1, my0, my1, mq0, mq1 = [], [], [], [], [], []
            _fine(do_plain(0, od), 4, end=False)
            stage((g_cp(2), w20), (x_cp(0), x_cp(2)))
            _fine(do_plain(2, od), 4, (g_forms(0, od), 72), (prep_b(0, 1, od), 7))
            stage((x_cp(0), x_cp(2)), (g_cp(1), g_cp(3), w10))
            xf = x_forms(0, od)
            _fine(stage_a(0, 0, (1,), mg0, od), 7, (_take(xf, 60), 60))
            stage((g_cp(1), g_cp(3), w10), (wqkv_cp, x_cp(1), x_cp(3)))
            _fine(_chain(do_plain(1, od), do_plain(3, od)), 8, (g_forms(1, od), 72), (_take(xf, 60), 60))
            _fine(stage_a(0, 1, (1,), mg1, od), 7, (xf, 72), (prep_b(0, 0, od), 7))
            stage((wqkv_cp, x_cp(1), x_cp(3)), w_cps(1))
            _fine(stage_a(0, 0, (0,), my0, od), 7,
                  (_chain(wqkv_t(od), w_forms(bq, lambda r: _bf(wqT[pl.ds(pl.multiple_of(r // 2 + z, 8), 24)]), HQ, od)), 14 + HQ // 48),
                  (prep_a(0, 0, od), 7))
            xf = x_forms(1, od)
            nx = 120
            pq, sg = proj(bq, rx[0], mq0, od), stage_g(0, 0, my0 + mg0, od, None)
            _fine(_take(pq, 3), 3, (_take(sg, 24), 24), (_take(xf, nx // 2), nx // 2))
            _fine(pq, 4, (sg, GU - 24), (_take(xf, nx // 2), nx // 2), (prep_a(0, 1, od), 7))
            _fine(stage_c(0, 0, True, od), 14, (xf, 192 - nx),
                  (_chain(finish_proj(0, mq0, qkv_place, od), grad_forms(0, g_rows, od)), 18 + 36))
            stage(w_cps(1), w_cps(2))
            _fine(stage_a(0, 1, (0,), my1, od), 7, (prep_a(1, 0, od), 7), (prep_a(1, 1, od), 7), (grad_forms(1, g_rows, od), 36), end=False)
            _fine(proj(bq, rx[1], mq1, od), 7, (stage_g(0, 1, my1 + mg1, od, None), GU), (grad_forms(1, x_rows, od), 36))
            _fine(stage_c(0, 1, True, od), 14, (_chain(finish_proj(1, mq1, qkv_place, od), grad_forms(0, x_rows, od)), 18 + 36),
                  (prep_b(1, 0, od), 7), (prep_b(1, 1, od), 7))

        pl.run_scoped(prologue, *[pltpu.VMEM((7, 192, CG), U32)] * 2,
                      pltpu.VMEM((7, HQ // 2, 384), U32), pltpu.VMEM((1, 2, D, 256), F32), pltpu.VMEM((3 * DP, 640), U32))

        def mlp_body(t, carry):
            i = t // 2
            j = t % 2

            def copies(_, c):
                @pl.when(jnp.logical_and(j == 0, i + 1 < NCH))
                def _():
                    for cp in w_cps(i + 1):
                        cp.wait()

                @pl.when(jnp.logical_and(j == 0, i + 2 < NCH))
                def _():
                    for cp in w_cps(i + 2):
                        cp.start()

                @pl.when(jnp.logical_and(j == 0, i >= 2))
                def _():
                    d_cp(i - 2, 1).start()
                    d_cp(i - 2, 0).wait()

                @pl.when(j == 1)
                def _():
                    d_cp(i - 1, 0).start()

                @pl.when(jnp.logical_and(j == 1, i >= 2))
                def _():
                    d_cp(i - 2, 1).wait()
                return c
            lax.fori_loop(0, z + 1, copies, 0)

            od = _Order(zero_s[0])
            m, n = [], []
            nxt = jnp.minimum(i + 1, NCH - 1)
            att = _chain(*[attn_stage2(jnp.minimum(NB + 2 - t, NB - 1), hg, od) for hg in range(4)],
                         *[attn_stage1(NB + 1 - t, hg, od) for hg in range(4)])
            na = 100
            _interleave(stage_a(i, j, (0, 1), m, od), 14, (_take(att, na), na), (prep_a(nxt, j, od), 7))

            lead = 2
            per = 10
            def after(u):
                if u < lead * 4:
                    return m[14 - lead + u // 4][(u % 4) * 128:(u % 4) * 128 + 8, 0:128]
                v = u - lead * 4
                r = ((v % per) * (HD // 8) // per) * 8
                return n[v // per][r:r + 8, 0:128]
            g = stage_g(i, j, m, od, after)
            e = stage_e(i - 1, j, n, od)
            left = GU
            for k in range(7):
                next(e)
                cnt = min(left, lead * 4 if k == 0 else per)
                for _ in range(cnt):
                    next(g)
                left -= cnt
            assert left == 0
            _interleave(stage_c(i, j, False, od), 14, (finish_e(j, n, od), 6), (att, 4 * (N1 + N2) - na), (prep_b(nxt, j, od), 7))

            return carry
        lax.fori_loop(2, NIT, mlp_body, 0)
        d_cp(NCH - 2, 1).start()

    V = pltpu.VMEM
    blocks = V((NB + 1, DP, 128), U32)
    pl.run_scoped(main_phase, V((2, 2, D, FC), BF), V((NCH, 8, FC), F32),
                  V((2, 7, CG // 2, 384), U32), V((2, 7, CG // 2, 384), U32), blocks, blocks, V((2, 7, CG // 2, HF), U32),
                  V((2, 2, 7, 192, HF), U32), V((2, 2, 7, HD // 2, HF), U32))

    def epilogue(gq, go, aq, ao, out_s, dx_s, dwqkv_s, dwo_s, dxb, dxc):
        def o_forms(od):
            for b in range(8):
                va, vb = _f(_bf(oT[b])), _f(_bf(oT[b + 8]))
                for k, v in enumerate(_beta_kr(va, vb, ones_pad)):
                    v = _words(v)
                    go[k, 0:KS[k] // 2, b * 128:(b + 1) * 128] = v
                    od.note_all(v, 64)
                yield 1

        def dq_forms(od):
            for b in range(7, -1, -1):
                for r in range(0, KQ // 2, 64):
                    nr = min(64, 3 * DP - KQ // 2 - r)
                    blocks = []
                    for r0, cnt in ((r, 64), (KQ // 2 + r, nr)):
                        for bb in (b, b + 8):
                            v = _f(_bf(dqkvT[bb, r0:r0 + cnt]))
                            blocks.append(v if cnt == 64 else _rows(v, zero_pad))
                    for k, v in enumerate(_beta(*blocks)):
                        v = _words(v)
                        gq[k, r:r + 64, b * 128:(b + 1) * 128] = v
                        od.note_all(v, 64)
                    yield 1

        def wq_forms(od):
            for r in range(0, HD, 48):
                u, l = _f(wqkv[r:r + 48]), _f(wqkv[HD + r:HD + r + 48])
                pad = jnp.zeros((48, 2 * KQ - 3 * D), F32)
                for k, v in enumerate(_alpha(u[:, :KQ], _cols(u[:, KQ:], pad), l[:, :KQ], _cols(l[:, KQ:], pad))):
                    v = _words(v)
                    aq[k, r // 2:r // 2 + 24] = v
                    od.note_all(v, 8)
                yield 1

        def wo_forms(od):
            rowd = lax.broadcasted_iota(jnp.int32, (64, D), 0)
            b2row = jnp.where(rowd == 0, jnp.broadcast_to(_f(b2_ref[...]).reshape(1, D), (64, D)), 0.0).astype(BF)
            woT = _rows(wo[...], b2row).T
            for r in range(0, HD, 48):
                u, l = _f(woT[r:r + 48]), _f(woT[HD + r:HD + r + 48])
                a = _alpha(u[:, 0:256], u[:, 256:512], l[:, 0:256], l[:, 256:512])
                ru, rl = u[:, 512:640], l[:, 512:640]
                forms = [a[0], a[1], _cols(a[2], ru), _cols(a[3], rl), a[4], _cols(a[5], rl - ru), _cols(a[6], ru - rl)]
                for k, v in enumerate(forms):
                    v = _words(v)
                    ao[k, r // 2:r // 2 + 24, 0:KS[k]] = v
                    od.note_all(v, 24)
                yield 1

        def o_cp(j):
            return pltpu.make_async_copy(out_s.at[j], outT_hbm.at[:, pl.ds(j * CG, CG)], sem_o.at[j])

        def dx_cp(j):
            return pltpu.make_async_copy(dx_s.at[j], dxT_hbm.at[:, pl.ds(j * CG, CG)], sem_dx.at[j])

        def ln2_bwd(j, od):
            for c in range(2):
                ls = slice(c * 256, (c + 1) * 256)
                st = {jj: [ln_s[jj, e, 0:1, ls] for e in range(4)] for jj in (j, j + 2)}

                def y(jj, r):
                    m1, r1, m2, r2 = st[jj]
                    return ((_f(xT[jj, r:r + 16, ls]) - _tile(od.gate(m1), 16)) * r1 - m2) * r2
                s1, s2 = {}, {}
                for r in range(0, HD, 16):
                    q = _combine([acc[0, j, k, r:r + 16, ls] for k in range(7)])
                    for jj, u, l in ((j, q[0], q[2]), (j + 2, q[1], q[3])):
                        dxb[jj, r:r + 16, ls] = u
                        dxb[jj, HD + r:HD + r + 16, ls] = l
                        v1, v2 = _fold(u + l), _fold(u * y(jj, r) + l * y(jj, HD + r))
                        s1[jj], s2[jj] = (v1, v2) if r == 0 else (s1[jj] + v1, s2[jj] + v2)
                        od.note(s1[jj], s2[jj])
                    yield 1
                a = {jj: (_mean(s1[jj]), _mean(s2[jj])) for jj in (j, j + 2)}
                for r in range(0, D, 32):
                    for jj in (j, j + 2):
                        for rr in (r, r + 16):
                            v = st[jj][3] * (dxb[jj + z, rr:rr + 16, ls] - _tile(od.gate(a[jj][0]), 16) - y(jj, rr) * a[jj][1])
                            dxc[jj, rr:rr + 16, ls] = v
                            od.note_all(pltpu.bitcast(v, U32), 16)
                    yield 1

        def out_proj(j, m, od):
            for k in range(7):
                m.append(od.dot(ao[k + z, :, 0:KS[k]], _bf(go[k + z, 0:KS[k] // 2, j * CG:(j + 1) * CG]), NN))
                yield 1

        def finish_out(j, m, od):
            for r in range(0, HD, 16):
                q = _combine([acc[1, j, k, r:r + 16] + m[k][r:r + 16] for k in range(7)])
                for jj, r0, v in ((j, r, q[0]), (j + 2, r, q[1]), (j, HD + r, q[2]), (j + 2, HD + r, q[3])):
                    v = (_f(xT[jj, r0:r0 + 16]) + v).astype(BF)
                    out_s[jj, r0:r0 + 16] = v
                    od.note(pltpu.bitcast(v, U32))
                yield 1

        def dx_proj(j, m, od):
            for k in range(7):
                m.append(od.dot(aq[k + z], _bf(gq[k + z, :, j * CG:(j + 1) * CG]), NN))
                yield 1

        def finish_dx(j, m, od):
            for r in range(0, HD, 16):
                q = _combine([v[r:r + 16] for v in m])
                for jj, r0, v in ((j, r, q[0]), (j + 2, r, q[1]), (j, HD + r, q[2]), (j + 2, HD + r, q[3])):
                    v = dxc[jj + z, r0:r0 + 16] + v
                    dxb[jj, r0:r0 + 16] = v
                    od.note_all(pltpu.bitcast(v, U32), 16)
                yield 1

        def ln1_bwd(j, od):
            m1, r1 = ln_s[j, 0, 0:1], ln_s[j, 1, 0:1]

            def xn(r):
                return (_f(xT[j, r:r + 32]) - m1) * r1
            s1 = s2 = None
            for r in range(0, D, 32):
                d = dxb[j + z, r:r + 32]
                v1, v2 = _fold(d), _fold(d * xn(r))
                s1, s2 = (v1, v2) if r == 0 else (s1 + v1, s2 + v2)
                od.note(s1, s2)
                yield 1
            a1, a2 = _mean(s1), _mean(s2)
            for r in range(0, D, 32):
                v = (_f(gT[j, r:r + 32]) + r1 * (dxb[j + z, r:r + 32] - a1 - xn(r) * a2)).astype(BF)
                dx_s[j, r:r + 32] = v
                od.note_all(pltpu.bitcast(v, U32), 8)
                yield 1

        def dwqkv_proj(c0, c1, n, od):
            for k in range(7):
                n.append(od.dot(tx[k], _bf(gq[k + z, c0 // 2:c1 // 2]), NT))
                yield 1

        def finish_dwqkv(c0, c1, n, od):
            c2 = min(c1, 3 * D - KQ)
            for r in range(0, HD, 16):
                q = _combine_t([v[r:r + 16] for v in n])
                for r0, u, l in ((r, q[0], q[1]), (HD + r, q[2], q[3])):
                    u, l = u.astype(BF), l.astype(BF)
                    dwqkv_s[r0:r0 + 16, c0:c1] = u
                    dwqkv_s[r0:r0 + 16, KQ + c0:KQ + c2] = l[:, 0:c2 - c0]
                    od.note(pltpu.bitcast(u, U32), pltpu.bitcast(l, U32))
                yield 1

        def dwo_proj(n, od):
            for k in range(7):
                n.append(od.dot(tg[1, k], _bf(go[k + z, 0:KS[k] // 2]), NT))
                yield 1

        def finish_dwo(n, od):
            q = _combine_t([v[:, 0:256] for v in n])
            ru = n[2][:, 256:] - n[5][:, 256:] + n[6][:, 256:]
            rl = n[3][:, 256:] + n[5][:, 256:] - n[6][:, 256:]
            t = _rows(_cols(q[0], q[1], ru), _cols(q[2], q[3], rl), jnp.zeros((64, 640), F32)).astype(BF).T
            dwo_s[...] = t[0:D, 0:D]
            db2_ref[...] = _f(t[D:D + 16, 0:D])[0:1].reshape(D).astype(BF)
            od.note_all(pltpu.bitcast(t, U32), 16)
            yield 1

        dwqkv_out = [pltpu.make_async_copy(dwqkv_s.at[:, c0:c1], dwqkv_hbm.at[:, c0:c1], sem_dw.at[u])
                     for u, (c0, c1) in enumerate(((0, 640), (KQ, KQ + 640), (640, KQ), (KQ + 640, 3 * D)))]
        dwo_out = pltpu.make_async_copy(dwo_s, dwo_hbm, sem_dw.at[4])
        od = _Order(zero_s[0])
        n1, n2, mo0, mo1, no, mx0, mx1, nq0, nq1 = [], [], [], [], [], [], [], [], []
        att = _chain(*[attn_stage2(0, hg, od) for hg in range(4)])
        dq, of, l0, l1 = dq_forms(od), o_forms(od), ln2_bwd(0, od), ln2_bwd(1, od)
        _fine(stage_e(NCH - 1, 0, n1, od), 7, (att, 4 * N2), (wo_forms(od), 6), (_take(of, 3), 3), end=False)
        for q in range(2):
            d_cp(NCH - 2, q).wait()
        _fine(stage_e(NCH - 1, 1, n2, od), 7, (finish_e(0, n1, od), 6), (of, 5), (_take(dq, 14), 14))
        d_cp(NCH - 1, 0).start()
        db1 = _cols(*[jnp.sum(db1s[i, 0] + db1s[i, 1], axis=0, keepdims=True) for i in range(NCH)])
        db1_ref[...] = db1.reshape(F).astype(BF)
        _fine(out_proj(0, mo0, od), 7, (finish_e(1, n2, od), 6), (_take(dq, 11), 11), end=False)
        d_cp(NCH - 1, 1).start()
        _fine(out_proj(1, mo1, od), 7, (finish_out(0, mo0, od), 18), (_take(dq, 11), 11))
        o_cp(0).start()
        o_cp(2).start()
        _fine(dwo_proj(no, od), 7, (finish_out(1, mo1, od), 18), (dq, 20), (wq_forms(od), 6))
        o_cp(1).start()
        o_cp(3).start()
        _fine(dx_proj(0, mx0, od), 7, (finish_dwo(no, od), 1), (l0, 72))
        dwo_out.start()
        _fine(dx_proj(1, mx1, od), 7, (finish_dx(0, mx0, od), 18), (l1, 72))
        _fine(dwqkv_proj(0, 640, nq0, od), 7,
              (_chain(ln1_bwd(0, od), ln1_bwd(2, od), finish_dx(1, mx1, od), ln1_bwd(1, od)), 3 * 36 + 18))
        for j in (0, 2, 1):
            dx_cp(j).start()
        last = dwqkv_proj(640, KQ, nq1, od)
        _fine(_take(last, 4), 4, (finish_dwqkv(0, 640, nq0, od), 18), (ln1_bwd(3, od), 36))
        for cp in (*dwqkv_out[0:2], dx_cp(3)):
            cp.start()
        _run(last)
        _run(finish_dwqkv(640, KQ, nq1, od))
        for cp in dwqkv_out[2:4]:
            cp.start()
        for q in range(2):
            d_cp(NCH - 1, q).wait()
        for j in range(NG):
            o_cp(j).wait()
            dx_cp(j).wait()
        for cp in dwqkv_out:
            cp.wait()
        dwo_out.wait()

    pl.run_scoped(epilogue, V((7, KQ // 2, HS), U32), V((7, 192, HS), U32), V((7, HD // 2, KQ), U32),
                  V((7, HD // 2, 384), U32), V((NG, D, CG), BF), V((NG, D, CG), BF), V((D, 3 * D), BF), V((D, D), BF),
                  V((NG, D, CG), F32), V((NG, D, CG), F32))


@jax.jit
def pallas_parallel_sum__sliding_local_dilated__mixer_channel_mlp__prompt_kernel(
    A_x, A_wqkv, A_wo, B_x, B_w1, B_b1, B_w2, B_b2, grad_out,
):
    del B_x
    hbm = pl.BlockSpec(memory_space=pl.ANY)
    vmem = pl.BlockSpec(memory_space=pltpu.VMEM)
    V = pltpu.VMEM
    dma = pltpu.SemaphoreType.DMA
    outs = pl.pallas_call(
        _kernel,
        in_specs=[hbm, hbm, hbm, hbm, hbm, vmem, hbm, vmem],
        out_specs=[hbm, hbm, hbm, hbm, hbm, vmem, hbm, vmem],
        out_shape=[
            jax.ShapeDtypeStruct((D, S), BF), jax.ShapeDtypeStruct((D, S), BF),
            jax.ShapeDtypeStruct((D, 3 * D), BF), jax.ShapeDtypeStruct((D, D), BF),
            jax.ShapeDtypeStruct((D, F), BF), jax.ShapeDtypeStruct((F,), BF),
            jax.ShapeDtypeStruct((D, F), BF), jax.ShapeDtypeStruct((D,), BF),
        ],
        scratch_shapes=[
            V((NG, D, CG), BF), V((NG, D, CG), BF), V((D, 3 * D), BF), V((D, D), BF),
            V((2, 7, HD // 2, HS), U32), V((7, HD // 2, HS), U32),
            V((NB, DP, 128), U32), V((NB, 3 * DP, 128), U32), V((2, 2, 7, HD, CG), F32),
            V((2, 2, 2, 7, CG // 2, HF), U32), V((NB + 1, DP, 128), U32), V((NB + 1, DP, 128), U32),
            V((4, W, H, 128), F32), V((4, W, H, 128), F32), V((NCH, 2, 8, FC), F32),
            V((NG, 4, 8, CG), F32),             V((2, 8, 128), U32), V((2, D, FC), BF),
            dma((NG,)), dma((NG,)), dma((5,)), dma((4,)), dma((2,)), dma((NG,)), dma((NG,)), dma((5,)),
        ],
        compiler_params=pltpu.CompilerParams(vmem_limit_bytes=128 * 2**20),
    )(A_x[0].T, grad_out[0].T, A_wqkv, A_wo, B_w1, B_b1, B_w2.T, B_b2)
    outT, dxT, dwqkv, dwo, dw1, db1, dw2T, db2 = outs
    return (outT.T[None], dxT.T[None], dwqkv, dwo, dw1, db1, dw2T.T, db2)
```

```python
import jax
import jax.numpy as jnp
from jax import lax
import jax.experimental.pallas as pl
import jax.experimental.pallas.tpu as pltpu

S, D, F = 2048, 576, 4608
H, DH, W, DIL = 32, 18, 8, 2
EPS = 1e-5
FC = 512
NCH = F // FC
CG = 512
NG = S // CG
NB = S // 128
DP = D // 2
HP = DH // 2
HG = 8
HF, HD, HS = FC // 2, D // 2, S // 2
NIT = 2 * NCH
HQ = 3 * HD
KQ = 896
KS = (256, 256, 384, 384, 256, 384, 384)
BF, F32, U32 = jnp.bfloat16, jnp.float32, jnp.uint32
C1 = 0.7978845608028654
C2 = C1 * 0.044715


NN = (((1,), (0,)), ((), ()))
NT = (((1,), (1,)), ((), ()))


def _dot(a, b, dn):
    return lax.dot_general(a, b, dn, preferred_element_type=F32)


def _f(v):
    return v.astype(F32)


def _words(v):
    return pltpu.bitcast(v.astype(BF), U32)


def _bf(t):
    return pltpu.bitcast(t, BF)


def _unpack(t):
    return pltpu.bitcast(t << 16, F32), pltpu.bitcast(t & jnp.uint32(0xFFFF0000), F32)


def _pack(lo, hi):
    lo = pltpu.bitcast(_f(lo.astype(BF)), U32) >> 16
    return lo | pltpu.bitcast(_f(hi.astype(BF)), U32)


def _alpha(a11, a12, a21, a22):
    return [a11 + a22, a21 + a22, a11, a22, a11 + a12, a21 - a11, a12 - a22]


def _beta(b11, b12, b21, b22):
    return [b11 + b22, b11, b12 - b22, b21 - b11, b22, b11 + b12, b21 + b22]


def _gamma(c11, c12, c21, c22):
    return [c11 + c22, c21 - c22, c12 + c22, c11 + c21, c12 - c11, c22, c11]


def _combine(m):
    return m[0] + m[3] - m[4] + m[6], m[2] + m[4], m[1] + m[3], m[0] - m[1] + m[2] + m[5]


def _combine_t(n):
    return n[0] + n[2] + n[4] - n[5], n[4] + n[6], n[1] + n[5], n[0] + n[1] + n[3] - n[6]


def _rows(*u):
    return jnp.concatenate(u, axis=0)


def _beta_kr(ta, tb, pad_a, pad_b):
    b = _beta(ta[0:256], tb[0:256], ta[256:512], tb[256:512])
    r1, r2 = _rows(ta[512:D], pad_a), _rows(tb[512:D], pad_b)
    return [b[0], b[1], _rows(b[2], r2), _rows(b[3], r1), b[4], _rows(b[5], r2), _rows(b[6], r1)]


def _cols(*u):
    return jnp.concatenate(u, axis=1)


def _word_forms(form, *words):
    vals = [_f(_bf(t)) for t in words]
    same = {id(v): t for v, t in zip(vals, words)}
    return [same[id(v)] if id(v) in same else _words(v) for v in form(*vals)]


def _lazy(form, *parts):
    class Term:
        def __init__(self, get):
            self.get = get

        def __add__(self, other):
            return Term(lambda: self.get() + other.get())

        def __sub__(self, other):
            return Term(lambda: self.get() - other.get())
    return [t.get for t in form(*[Term(p) for p in parts])]


def _alpha_k_tiles(ga, gb, pad):
    out = []
    for t in range(2):
        r = t * 128
        forms = _lazy(_alpha, lambda r=r: ga(r, 128), lambda r=r: ga(256 + r, 128),
                      lambda r=r: gb(r, 128), lambda r=r: gb(256 + r, 128))
        out += [(k, t, v) for k, v in enumerate(forms)]
    zero = jnp.zeros_like(pad)
    out += [(2, 2, lambda: _rows(ga(512, 64), pad)), (3, 2, lambda: _rows(gb(512, 64), pad)),
            (5, 2, lambda: _rows(gb(512, 64) - ga(512, 64), zero)), (6, 2, lambda: _rows(ga(512, 64) - gb(512, 64), zero))]
    return out


def _tile(v, n):
    return _rows(*[v] * (n // 8))


def _fold(v):
    return jnp.sum(v.reshape(v.shape[0] // 8, 8, v.shape[1]), axis=0)


def _mean(part):
    return jnp.sum(part, axis=0, keepdims=True) * (1.0 / D)


def _gelu(pre, dh, c2):
    x2c = (c2 * pre) * pre
    ht = 0.5 * jnp.tanh(pre * (C1 + x2c))
    sg = 0.5 + ht
    h = pre * sg
    return h, dh * (sg + h * (0.5 - ht) * (2.0 * C1 + 6.0 * x2c))


def _interleave(od, main, n_main, *side, head=0):
    done = [0] * len(side)
    for k in range(n_main):
        for q, (gen, n) in enumerate(side):
            while done[q] < ((2 * k + head) * n) // (2 * n_main - 2 + head):
                next(gen)
                done[q] += 1
        if k == 0:
            od.pending = [None] * len(od.pending) + od.pending
        next(main)
    for gen in (main, *[g for g, _ in side]):
        assert next(gen, None) is None


def _chain(*gens):
    for g in gens:
        yield from g


def _take(gen, n):
    for _ in range(n):
        yield next(gen)


def _run(gen):
    for _ in gen:
        pass


class _Order:
    def __init__(self, zero):
        self.zero = zero
        self.pending = []
        self.last = None

    def note(self, *vs):
        vs = [v if v.dtype == U32 else pltpu.bitcast(v, U32) for v in vs]
        vs = [v[:, c:c + 128] for v in vs for c in range(0, v.shape[1], 128)]
        out = vs[0]
        for v in vs[1:]:
            out = out | v
        self.pending.append(out)

    def note_all(self, v, n=4):
        regs = [v[r:r + 8, c:c + 128] for r in range(0, v.shape[0], 8) for c in range(0, v.shape[1] - 127, 128)]
        for e in range(0, len(regs), n):
            self.note(*regs[e:e + n])

    def dot(self, a, b, dn):
        ax = 1 if dn == NN else 0
        width = 128 if a.shape[1] >= 512 else 256
        blocks = [(c, min(c + width, b.shape[ax])) for c in range(0, b.shape[ax], width)]
        slots = [(u, kc, r) for u in range(len(blocks)) for kc in range(0, a.shape[1] - 127, 512)
                 for r in range(0, a.shape[0], 8)]
        at = {}
        for q, v in enumerate(self.pending):
            key = slots[q * len(slots) // len(self.pending)]
            if v is not None:
                at[key] = v if key not in at else at[key] | v
        self.pending = []
        out = []
        for u, (c0, c1) in enumerate(blocks):
            parts, prev = [], 0
            for r in sorted({r for (uu, _, r) in at if uu == u}):
                if r > prev:
                    parts.append(a[prev:r])
                row, pc = [], 0
                for kc in range(0, a.shape[1] - 127, 512):
                    if (u, kc, r) in at:
                        if kc > pc:
                            row.append(a[r:r + 8, pc:kc])
                        row.append(a[r:r + 8, kc:kc + 128] | (at[u, kc, r] & self.zero))
                        pc = kc + 128
                if pc < a.shape[1]:
                    row.append(a[r:r + 8, pc:])
                parts.append(_cols(*row))
                prev = r + 8
            if prev < a.shape[0]:
                parts.append(a[prev:])
            out.append(_dot(_bf(_rows(*parts)), b[:, c0:c1] if ax else b[c0:c1], dn))
        self.last, self.calls = out[-1], 0
        if a.shape[0] > CG // 2:
            self.last = _rows(*[v[:, 0:128] for v in out])
        return _cols(*out)

    def hold(self, t, after=None):
        if after is None:
            if self.last is None:
                return t
            rows = self.last.shape[0]
            step = 40 if rows < CG else 56 if rows == CG else 144
            r = min(self.calls * step, self.last.shape[0] - 8)
            self.calls += 1
            after = self.last[r:r + 8, 0:128]
        return t | (pltpu.bitcast(after, U32) & self.zero)

    def gate(self, v):
        v = pltpu.bitcast(jnp.broadcast_to(v, (8, v.shape[1])), U32)
        if self.last is not None:
            u = pltpu.bitcast(self.last[0:8, 0:128], U32) & self.zero
            v = v | _cols(*[u] * (v.shape[1] // 128))
        return pltpu.bitcast(v, F32)


def _kernel(xT_hbm, gT_hbm, wqkv_hbm, wo_hbm, w1_hbm, b1_ref, w2T_hbm, b2_ref,
            outT_hbm, dxT_hbm, dwqkv_hbm, dwo_hbm, dw1_hbm, db1_ref, dw2T_hbm, db2_ref,
            xT, gT, wqkv, wo, tg, tx, oT, dqkvT, acc, hf, qT, doT, p_s, ds_s, db1s, ln_s, zero_s, dw_s,
            sem_x, sem_g, sem_w, sem_wc, sem_d, sem_o, sem_dx, sem_dw):

    def x_cp(j):
        return pltpu.make_async_copy(xT_hbm.at[:, pl.ds(j * CG, CG)], xT.at[j], sem_x.at[j])

    def g_cp(j):
        return pltpu.make_async_copy(gT_hbm.at[:, pl.ds(j * CG, CG)], gT.at[j], sem_g.at[j])

    def chunk(i):
        return pl.ds(i * FC if isinstance(i, int) else pl.multiple_of(i * FC, FC), FC)

    def d_cp(i, q):
        return pltpu.make_async_copy(dw_s.at[q], (dw1_hbm, dw2T_hbm)[q].at[:, chunk(i)], sem_d.at[q])

    wo_cp = [pltpu.make_async_copy(wo_hbm.at[r:r + 144], wo.at[r:r + 144], sem_w.at[r // 144]) for r in range(0, D, 144)]
    wqkv_cp = pltpu.make_async_copy(wqkv_hbm, wqkv, sem_w.at[4])
    rowp = lax.broadcasted_iota(jnp.int32, (64, 128), 0)
    ones_pad = jnp.where(rowp == 0, 1.0, 0.0)
    zero_pad = jnp.zeros((64, 128), F32)

    def clear(i, carry):
        zero_s[i] = jnp.zeros((8, 128), U32)
        return carry + i
    z = lax.fori_loop(0, 2, clear, -1)

    def fence():
        lax.fori_loop(1, z + 2, clear, 0)

    def _segment(od, main, n_main, *side, end=True):
        _interleave(od, main, n_main, *side, head=1)
        if end:
            fence()

    def zz(j):
        return z if isinstance(j, int) else 0

    scale = DH ** -0.5
    lane = lax.broadcasted_iota(jnp.int32, (HG, 128), 1)

    def back(prev, cur, w):
        if w == 0:
            return cur
        return pltpu.roll(jnp.where(lane >= 128 - DIL * w, prev, cur), DIL * w, 1)

    def fwd(cur, nxt, w):
        if w == 0:
            return cur
        return pltpu.roll(jnp.where(lane < DIL * w, nxt, cur), 128 - DIL * w, 1)

    def attn_stage2(c, hg, od):
        hs = pl.ds(hg * HG, HG)
        c = c + zz(c)
        for src, wt, off in ((qT, ds_s, DP), (doT, p_s, 2 * DP)):
            ws = [fwd(wt[c % 4, w, hs, :], wt[(c + 1) % 4, w, hs, :], w) for w in range(W)]
            for d in range(HP):
                rows = pl.ds(hg * HG * HP + d, HG, stride=HP)
                sc, sn = src[c, rows, :], src[c + 1, rows, :]
                sc = od.hold(sc)
                al = ah = None
                for w in range(W):
                    sl, sh = _unpack(fwd(sc, sn, w))
                    al = ws[w] * sl if w == 0 else al + ws[w] * sl
                    ah = ws[w] * sh if w == 0 else ah + ws[w] * sh
                res = _pack(al, ah)
                dst = pl.ds(off + hg * HG * HP + d, HG, stride=HP)
                dqkvT[c, dst, :] = res
                od.note(res)
                yield 1

    N1, N2 = 3 * HP + 1, 2 * HP

    def stage_e(i, q, out, od):
        for k in range(7):
            out.append(od.dot(tg[q, k], _bf(_rows(hf[i % 2, 0, q, k], hf[i % 2, 1, q, k])), NN))
            yield 1

    def finish_e(q, n, od):
        for r in range(0, HD, 48):
            for v, (r0, c0) in zip(_combine_t([u[r:r + 48] for u in n]), ((0, 0), (0, HF), (HD, 0), (HD, HF))):
                v = v.astype(BF)
                dw_s[q, r0 + r:r0 + r + 48, c0:c0 + HF] = v
                od.note_all(pltpu.bitcast(v, U32), n=2)
            yield 1

    def main_phase(wc, b1s, ta0, ta1, kT, vT, hx, bf, af):
        ta = (ta0, ta1)

        def w_cps(i):
            return [pltpu.make_async_copy(src.at[:, chunk(i)], wc.at[i % 2, q], sem_wc.at[2 * (i % 2) + q])
                    for q, src in enumerate((w1_hbm, w2T_hbm))]

        def attn_stage1(c, hg, od):
            def rows(d):
                return pl.ds(hg * HG * HP + d, HG, stride=HP)
            hs = pl.ds(hg * HG, HG)
            lg = [None] * W
            c = c + zz(c)
            for d in range(HP):
                ql, qh = _unpack(qT[c, rows(d), :])
                kp, kc = kT[c, rows(d), :], kT[c + 1, rows(d), :]
                kc = od.hold(kc)
                for w in range(W):
                    kl, kh = _unpack(back(kp, kc, w))
                    t = ql * kl + qh * kh
                    lg[w] = t if d == 0 else lg[w] + t
                od.note(*lg)
                yield 1
            tok = lane + c * 128
            lg = [lg[0] * scale] + [jnp.where(tok >= DIL * w, lg[w] * scale, -1e9) for w in range(1, W)]
            m = lg[0]
            for w in range(1, W):
                m = jnp.maximum(m, lg[w])
            e = [jnp.exp(l - m) for l in lg]
            tot = e[0]
            for w in range(1, W):
                tot = tot + e[w]
            inv = 1.0 / tot
            p = [x * inv for x in e]
            od.note(inv)
            yield 1
            dp = [None] * W
            for d in range(HP):
                gl, gh = _unpack(doT[c, rows(d), :])
                vp, vc = vT[c, rows(d), :], vT[c + 1, rows(d), :]
                vc = od.hold(vc)
                ol = oh = None
                for w in range(W):
                    vl, vh = _unpack(back(vp, vc, w))
                    t = gl * vl + gh * vh
                    dp[w] = t if d == 0 else dp[w] + t
                    ol = p[w] * vl if w == 0 else ol + p[w] * vl
                    oh = p[w] * vh if w == 0 else oh + p[w] * vh
                res = _pack(ol, oh)
                oT[c, rows(d), :] = res
                od.note(res, *dp)
                yield 1
            dot = p[0] * dp[0]
            for w in range(1, W):
                dot = dot + p[w] * dp[w]
            ds = [p[w] * (dp[w] - dot) * scale for w in range(W)]
            od.note(dot)
            for w in range(W):
                p_s[c % 4, w, hs, :] = p[w]
                ds_s[c % 4, w, hs, :] = ds[w]
            for d in range(HP):
                kp, kc = kT[c, rows(d), :], kT[c + 1, rows(d), :]
                kc = od.hold(kc)
                al = ah = None
                for w in range(W):
                    kl, kh = _unpack(back(kp, kc, w))
                    al = ds[w] * kl if w == 0 else al + ds[w] * kl
                    ah = ds[w] * kh if w == 0 else ah + ds[w] * kh
                res = _pack(al, ah)
                dqkvT[c, rows(d), :] = res
                od.note(res)
                yield 1

        row64 = lax.broadcasted_iota(jnp.int32, (64, FC), 0)

        def put(dst, forms, od):
            for k, v in enumerate(forms):
                v = _words(v)
                dst[k, 0:v.shape[0]] = v
                od.note_all(v, n=6)
                yield 1

        def prep_b(i, q, od):
            w = _f(wc[i % 2, q])
            brow = jnp.where(jnp.logical_and(row64 == 0, q == 0), jnp.broadcast_to(b1s[i][0:1], (64, FC)), 0.0)
            yield from put(bf.at[i % 2, q], _beta_kr(w[:, :HF], w[:, HF:], brow[:, :HF], brow[:, HF:]), od)

        def prep_a(i, q, od):
            w = _f(wc[i % 2, q])
            yield from put(af.at[i % 2, q], _alpha(w[0:HD, :HF], w[0:HD, HF:], w[HD:D, :HF], w[HD:D, HF:]), od)

        def stage_a(i, j, qs, out, od):
            for q in qs:
                for k in range(7):
                    out.append(od.dot(ta[q][j + zz(j), k, :, 0:KS[k]], _bf(bf[i % 2 + zz(j), q, k, 0:KS[k] // 2]), NN))
                    yield 1

        GU = (CG // 16) * (HF // 128)

        def stage_g(i, j, m, od, after):
            sums = {}
            for u in range(GU):
                r, c = (u // 2) * 16, (u % 2) * 128
                pre = _combine([v[r:r + 16, c:c + 128] for v in m[0:7]])
                dh = _combine([v[r:r + 16, c:c + 128] for v in m[7:14]])
                c2 = pltpu.bitcast(jnp.full((8, 128), C2, F32), U32)
                c2 = pltpu.bitcast(od.hold(c2, None if after is None else after(u)), F32)
                c2 = _rows(c2, c2)
                hd = [_gelu(p_, q_, c2) for p_, q_ in zip(pre, dh)]
                done = []
                for q in range(2):
                    h11, h12, h21, h22 = [v[1 - q] for v in hd]
                    for k, v in enumerate(_beta(h11, h21, h12, h22)):
                        v = _words(v)
                        hx[q, k, r // 2:r // 2 + 8, c:c + 128] = v
                        done.append(v)
                done = done[7:] + done[:7]
                for e in range(0, 14, 3):
                    od.note(*done[e:e + 3])
                for col, v in ((c, hd[0][1] + hd[2][1]), (HF + c, hd[1][1] + hd[3][1])):
                    v = v[0:8] + v[8:16]
                    sums[col] = v if col not in sums else sums[col] + v
                if u == GU - 1:
                    for col, v in sums.items():
                        db1s[i, j, :, col:col + 128] = v
                yield 1

        def stage_c(i, j, first, od):
            for q in (1, 0):
                for k in range(7):
                    v = hx[q + z, k]
                    hf[i % 2, j, q, k] = v
                    r = od.dot(af[i % 2 + zz(j), q, k], _bf(v), NT)
                    acc[q, j, k] = r if first else acc[q, j, k] + r
                    yield 1

        def init():
            zero_blk = jnp.zeros((DP, 128), U32)
            kT[0] = zero_blk
            vT[0] = zero_blk
            qT[NB] = zero_blk
            doT[NB] = zero_blk
            for blk in (NB - 1, NB):
                p_s[blk % 4] = jnp.zeros((W, H, 128), F32)
                ds_s[blk % 4] = jnp.zeros((W, H, 128), F32)
            b1f32 = _f(b1_ref[...]).reshape(1, F)
            for i in range(NCH):
                b1s[i] = jnp.broadcast_to(b1f32[:, i * FC:(i + 1) * FC], (8, FC))

        def prologue(rx0, rx1, bq, lnb, wqT):
            rx = (rx0, rx1)

            def tok_forms(j, c, ga, gb, pad, nat, raw, od):
                for k, t, get in _alpha_k_tiles(ga, gb, pad):
                    v = get().astype(BF)
                    if raw is not None:
                        u = pltpu.bitcast(v, U32)
                        raw[k, t * 64:(t + 1) * 64, c * 128:(c + 1) * 128] = u
                    if nat is not None:
                        u = pltpu.bitcast(v.T, U32)
                        nat[j, k, c * 64:(c + 1) * 64, t * 128:(t + 1) * 128] = u
                    od.note_all(u)
                    yield 1

            def g_forms(j, od):
                for c in range(4):
                    ls = slice(c * 128, (c + 1) * 128)
                    yield from tok_forms(j, c, lambda r, n: _f(gT[j, r:r + n, ls]), lambda r, n: _f(gT[j + 2, r:r + n, ls]),
                                         zero_pad, ta[1], None, od)

            def grad_forms(j, get, od):
                for r in range(0, HD, 16):
                    for c in range(0, CG, 256):
                        ls = slice(c, c + 256)
                        for blocks in zip(get(j, r, ls), get(j + 2, r, ls), get(j, HD + r, ls), get(j + 2, HD + r, ls)):
                            done = [_words(v) for v in _gamma(*[v for _, v in blocks])]
                            for k, v in enumerate(done):
                                blocks[0][0][k, r // 2:r // 2 + 8, j * CG + c:j * CG + c + 256] = v
                            od.note_all(_cols(*done[0:5]))
                        yield 1

            def g_rows(jj, r, ls):
                return [(tg.at[1], _f(gT[jj, r:r + 16, ls]))]

            def x_rows(jj, r, ls):
                m1, r1, m2, r2 = [ln_s[jj + z, e, 0:1, ls] for e in range(4)]
                xn = (_f(xT[jj, r:r + 16, ls]) - m1) * r1
                return [(tx, xn), (tg.at[0], (xn - m2) * r2)]

            def x_forms(j, od):
                for c in range(2):
                    ls = slice(c * 256, (c + 1) * 256)

                    def sweep(term):
                        tot = None
                        for r in range(0, D, 96):
                            v = [_fold(term(u, r)) for u in range(2)]
                            tot = v if tot is None else [tot[u] + v[u] for u in range(2)]
                            od.note(*tot)
                            yield 1
                        return [_mean(v) for v in tot]

                    def x(u, r):
                        return _f(xT[j + 2 * u, r:r + 96, ls])

                    def xn_new(u, r):
                        v = (x(u, r) - m1[u]) * r1[u]
                        lnb[0, u, r:r + 96] = v
                        return v

                    def xn(u, r):
                        return lnb[z, u, r:r + 96]
                    m1 = yield from sweep(x)
                    r1 = [lax.rsqrt(v + EPS) for v in (yield from sweep(lambda u, r: jnp.square(x(u, r) - m1[u])))]
                    m2 = yield from sweep(xn_new)
                    r2 = [lax.rsqrt(v + EPS) for v in (yield from sweep(lambda u, r: jnp.square(xn(u, r) - m2[u])))]
                    for u in range(2):
                        for e, v in enumerate((m1, r1, m2, r2)):
                            ln_s[j + 2 * u, e, :, ls] = jnp.broadcast_to(v[u], (8, 256))
                    for b in range(2):
                        bs = slice(b * 128, (b + 1) * 128)
                        xa, xb = [lambda r, n, u=u: lnb[z, u, r:r + n, bs] for u in range(2)]
                        ya, yb = [lambda r, n, u=u: (lnb[z, u, r:r + n, bs] - m2[u][:, bs]) * r2[u][:, bs] for u in range(2)]
                        yield from tok_forms(j, 2 * c + b, ya, yb, ones_pad, ta[0], None, od)
                        yield from tok_forms(j, 2 * c + b, xa, xb, zero_pad, None, rx[j], od)

            def wqkv_t(od):
                for c in range(0, 3 * D, 128):
                    n = min(128, 3 * D - c)
                    v = _rows(wqkv[:, c:c + n], jnp.zeros((64, n), BF)).T
                    wqT[c // 2:(c + n) // 2] = u = pltpu.bitcast(v, U32)
                    od.note_all(u)
                    yield 1

            def w_forms(dst, w, n, od):
                for r in range(0, n, 16):
                    u, l = _f(w(r)), _f(w(n + r))
                    b = _beta(u[:, 0:256], l[:, 0:256], u[:, 256:512], l[:, 256:512])
                    r1, r2 = u[:, 512:640], l[:, 512:640]
                    forms = [b[0], b[1], _cols(b[2], r2), _cols(b[3], r1), b[4], _cols(b[5], r2), _cols(b[6], r1)]
                    for k, v in enumerate(forms):
                        v = _words(v)
                        dst[k, r // 2:r // 2 + 8, 0:KS[k]] = v
                        od.note_all(v)
                    yield 1

            def proj(wf, src, m, od):
                for k in range(7):
                    m.append(od.dot(wf[k + z, :, 0:KS[k]], _bf(src[k + z, 0:KS[k] // 2]), NN))
                    yield 1

            def finish_proj(j, m, place, od):
                n = m[0].shape[0]
                for r in range(0, n, 16):
                    q = _combine([v[r:r + 16] for v in m])
                    for jj, r0, v in ((j, r, q[0]), (j, n + r, q[1]), (j + 2, r, q[2]), (j + 2, n + r, q[3])):
                        v = _words(v)
                        ref, shift, row = place(r0 // 2)
                        for b in range(4):
                            ref[jj * 4 + b + shift, row:row + 8] = v[:, b * 128:(b + 1) * 128]
                        od.note_all(v)
                    yield 1

            def qkv_place(r):
                return ((qT, 0), (kT, 1), (vT, 1))[r // DP] + (r % DP,)

            def do_plain(j, od):
                for r in range(0, D, 144):
                    if j == 0:
                        wo_cp[r // 144].wait()
                    v = _words(od.dot(pltpu.bitcast(wo[r:r + 144], U32), gT[j], NN))
                    for b in range(4):
                        doT[j * 4 + b, r // 2:r // 2 + 72] = v[:, b * 128:(b + 1) * 128]
                    yield 1

            def stage(wait, start):
                for cp in wait:
                    cp.wait()
                for cp in start:
                    cp.start()

            w10, w20 = w_cps(0)
            stage((), (g_cp(0), wo_cp[0]))
            init()
            stage((), wo_cp[1:])
            stage((g_cp(0),), (g_cp(2), w20))
            od = _Order(zero_s[0])
            mg0, mg1, my0, my1, mq0, mq1 = [], [], [], [], [], []
            _segment(od, do_plain(0, od), 4, end=False)
            stage((g_cp(2), w20), (x_cp(0), x_cp(2)))
            _segment(od, do_plain(2, od), 4, (g_forms(0, od), 72), (prep_b(0, 1, od), 7))
            stage((x_cp(0), x_cp(2)), (g_cp(1), g_cp(3), w10))
            xf = x_forms(0, od)
            _segment(od, stage_a(0, 0, (1,), mg0, od), 7, (_take(xf, 60), 60))
            stage((g_cp(1), g_cp(3), w10), (wqkv_cp, x_cp(1), x_cp(3)))
            _segment(od, _chain(do_plain(1, od), do_plain(3, od)), 8, (g_forms(1, od), 72), (_take(xf, 60), 60))
            _segment(od, stage_a(0, 1, (1,), mg1, od), 7, (xf, 72), (prep_b(0, 0, od), 7))
            stage((wqkv_cp, x_cp(1), x_cp(3)), w_cps(1))
            _segment(od, stage_a(0, 0, (0,), my0, od), 7,
                  (_chain(wqkv_t(od), w_forms(bq, lambda r: _bf(wqT[pl.ds(pl.multiple_of(r // 2 + z, 8), 8)]), HQ, od)), 14 + HQ // 16))
            xf = x_forms(1, od)
            nx = 80
            pq, sg = proj(bq, rx[0], mq0, od), stage_g(0, 0, my0 + mg0, od, None)
            _segment(od, _take(pq, 3), 3, (_take(sg, 24), 24), (_take(xf, nx // 2), nx // 2), (prep_a(0, 0, od), 7))
            _segment(od, pq, 4, (sg, GU - 24), (_take(xf, nx // 2), nx // 2), (prep_a(0, 1, od), 7))
            _segment(od, stage_c(0, 0, True, od), 14, (xf, 192 - nx),
                  (finish_proj(0, mq0, qkv_place, od), 54))
            stage(w_cps(1), w_cps(2))
            _segment(od, stage_a(0, 1, (0,), my1, od), 7, (prep_a(1, 0, od), 7), (prep_a(1, 1, od), 7), (grad_forms(0, g_rows, od), 36), end=False)
            _segment(od, proj(bq, rx[1], mq1, od), 7, (stage_g(0, 1, my1 + mg1, od, None), GU), (grad_forms(1, x_rows, od), 36))
            _segment(od, stage_c(0, 1, True, od), 14, (_chain(finish_proj(1, mq1, qkv_place, od), grad_forms(0, x_rows, od)), 54 + 36), (grad_forms(1, g_rows, od), 36),
                  (prep_b(1, 0, od), 7), (prep_b(1, 1, od), 7))

        pl.run_scoped(prologue, *[pltpu.VMEM((7, 192, CG), U32)] * 2,
                      pltpu.VMEM((7, HQ // 2, 384), U32), pltpu.VMEM((1, 2, D, 256), F32), pltpu.VMEM((3 * DP, 640), U32))

        def mlp_body(t, carry):
            i = t // 2
            j = t % 2

            def copies(_, c):
                @pl.when(j == 0)
                def _():
                    @pl.when(i + 1 < NCH)
                    def _():
                        for cp in w_cps(i + 1):
                            cp.wait()

                    @pl.when(i + 2 < NCH)
                    def _():
                        for cp in w_cps(i + 2):
                            cp.start()

                    @pl.when(i >= 2)
                    def _():
                        d_cp(i - 2, 1).start()
                        d_cp(i - 2, 0).wait()

                @pl.when(j == 1)
                def _():
                    d_cp(i - 1, 0).start()

                    @pl.when(i >= 2)
                    def _():
                        d_cp(i - 2, 1).wait()
                return c
            lax.fori_loop(0, z + 1, copies, 0)

            od = _Order(zero_s[0])
            m, n = [], []
            nxt = jnp.minimum(i + 1, NCH - 1)
            att = _chain(*[attn_stage2(jnp.minimum(NB + 2 - t, NB - 1), hg, od) for hg in range(H // HG)],
                         *[attn_stage1(NB + 1 - t, hg, od) for hg in range(H // HG)])
            na = 108
            _interleave(od, stage_a(i, j, (0, 1), m, od), 14, (_take(att, na), na), (prep_a(nxt, j, od), 7))

            lead = 2
            per = 10

            def after(u):
                if u < lead * 4:
                    return m[14 - lead + u // 4][(u % 4) * 128:(u % 4) * 128 + 8, 0:128]
                v = u - lead * 4
                r = ((v % per) * (HD // 4) // per) * 8
                return n[v // per][r % HD:r % HD + 8, (r // HD) * 128:(r // HD) * 128 + 128]
            g = stage_g(i, j, m, od, after)
            e = stage_e(i - 1, j, n, od)
            left = GU
            for k in range(7):
                next(e)
                cnt = min(left, lead * 4 if k == 0 else per)
                for _ in range(cnt):
                    next(g)
                left -= cnt
            assert left == 0
            _interleave(od, stage_c(i, j, False, od), 14, (finish_e(j, n, od), 6), (att, 4 * (N1 + N2) - na), (prep_b(nxt, j, od), 7))

            return carry
        lax.fori_loop(2, NIT, mlp_body, 0)
        d_cp(NCH - 2, 1).start()

    V = pltpu.VMEM
    blocks = V((NB + 1, DP, 128), U32)
    pl.run_scoped(main_phase, V((2, 2, D, FC), BF), V((NCH, 8, FC), F32),
                  V((2, 7, CG // 2, 384), U32), V((2, 7, CG // 2, 384), U32), blocks, blocks, V((2, 7, CG // 2, HF), U32),
                  V((2, 2, 7, 192, HF), U32), V((2, 2, 7, HD // 2, HF), U32))

    def epilogue(gq, go, aq, ao, out_s, dx_s, dwqkv_s, dwo_s, dxb, dxc):
        def o_forms(od):
            for b in range(8):
                ls = slice(b * 128, (b + 1) * 128)
                for r in range(0, 128, 32):
                    blocks = [oT[bb, r0:r0 + 32] for r0 in (r, 128 + r) for bb in (b, b + 8)]
                    for k, v in enumerate(_word_forms(_beta, *blocks)):
                        go[k, r:r + 32, ls] = v
                        if k not in (1, 4):
                            od.note_all(v)
                    yield 1
                for k, bb in ((2, b + 8), (3, b), (5, b + 8), (6, b)):
                    go[k, 128:192, ls] = _rows(oT[bb, 256:DP], _words(ones_pad))
                yield 1

        def dq_forms(od):
            for b in range(7, -1, -1):
                for r in range(0, KQ // 2, 64):
                    nr = min(64, 3 * DP - KQ // 2 - r)
                    blocks = []
                    for r0, cnt in ((r, 64), (KQ // 2 + r, nr)):
                        for bb in (b, b + 8):
                            v = dqkvT[bb, r0:r0 + cnt]
                            blocks.append(v if cnt == 64 else _rows(v, jnp.zeros((64 - cnt, 128), U32)))
                    for k, v in enumerate(_word_forms(_beta, *blocks)):
                        gq[k, r:r + 64, b * 128:(b + 1) * 128] = v
                        if k not in (1, 4):
                            od.note_all(v)
                    yield 1

        def wq_forms(od):
            for r in range(0, HD, 16):
                u, l = _f(wqkv[r:r + 16]), _f(wqkv[HD + r:HD + r + 16])
                pad = jnp.zeros((16, 2 * KQ - 3 * D), F32)
                for k, v in enumerate(_alpha(u[:, :KQ], _cols(u[:, KQ:], pad), l[:, :KQ], _cols(l[:, KQ:], pad))):
                    v = _words(v)
                    aq[k, r // 2:r // 2 + 8] = v
                    od.note_all(v)
                yield 1

        def wo_forms(od):
            rowd = lax.broadcasted_iota(jnp.int32, (64, D), 0)
            b2row = jnp.where(rowd == 0, jnp.broadcast_to(_f(b2_ref[...]).reshape(1, D), (64, D)), 0.0).astype(BF)
            woT = _rows(wo[...], b2row).T
            for r in range(0, HD, 16):
                u, l = _f(woT[r:r + 16]), _f(woT[HD + r:HD + r + 16])
                a = _alpha(u[:, 0:256], u[:, 256:512], l[:, 0:256], l[:, 256:512])
                ru, rl = u[:, 512:640], l[:, 512:640]
                forms = [a[0], a[1], _cols(a[2], ru), _cols(a[3], rl), a[4], _cols(a[5], rl - ru), _cols(a[6], ru - rl)]
                for k, v in enumerate(forms):
                    v = _words(v)
                    ao[k, r // 2:r // 2 + 8, 0:KS[k]] = v
                    od.note_all(v)
                yield 1

        def o_cp(j):
            return pltpu.make_async_copy(out_s.at[j], outT_hbm.at[:, pl.ds(j * CG, CG)], sem_o.at[j])

        def dx_cp(j):
            return pltpu.make_async_copy(dx_s.at[j], dxT_hbm.at[:, pl.ds(j * CG, CG)], sem_dx.at[j])

        def ln2_bwd(j, od):
            for c in range(2):
                ls = slice(c * 256, (c + 1) * 256)
                st = {jj: [ln_s[jj, e, 0:1, ls] for e in range(4)] for jj in (j, j + 2)}

                def y(jj, r):
                    m1, r1, m2, r2 = st[jj]
                    return ((_f(xT[jj, r:r + 16, ls]) - _tile(od.gate(m1), 16)) * r1 - m2) * r2
                s1, s2 = {}, {}
                for r in range(0, HD, 16):
                    q = _combine([acc[0, j, k, r:r + 16, ls] for k in range(7)])
                    for jj, u, l in ((j, q[0], q[2]), (j + 2, q[1], q[3])):
                        dxb[jj, r:r + 16, ls] = u
                        dxb[jj, HD + r:HD + r + 16, ls] = l
                        v1, v2 = _fold(u + l), _fold(u * y(jj, r) + l * y(jj, HD + r))
                        s1[jj], s2[jj] = (v1, v2) if r == 0 else (s1[jj] + v1, s2[jj] + v2)
                        od.note(s1[jj], s2[jj])
                    yield 1
                a = {jj: (_mean(s1[jj]), _mean(s2[jj])) for jj in (j, j + 2)}
                for r in range(0, D, 32):
                    for jj in (j, j + 2):
                        for rr in (r, r + 16):
                            v = st[jj][3] * (dxb[jj + z, rr:rr + 16, ls] - _tile(od.gate(a[jj][0]), 16) - y(jj, rr) * a[jj][1])
                            dxc[jj, rr:rr + 16, ls] = v
                            od.note_all(pltpu.bitcast(v, U32))
                    yield 1

        def out_proj(j, m, od):
            for k in range(7):
                m.append(od.dot(ao[k + z, :, 0:KS[k]], _bf(go[k + z, 0:KS[k] // 2, j * CG:(j + 1) * CG]), NN))
                yield 1

        def finish_out(j, m, od):
            for r in range(0, HD, 16):
                q = _combine([acc[1, j, k, r:r + 16] + m[k][r:r + 16] for k in range(7)])
                for jj, r0, v in ((j, r, q[0]), (j + 2, r, q[1]), (j, HD + r, q[2]), (j + 2, HD + r, q[3])):
                    v = (_f(xT[jj, r0:r0 + 16]) + v).astype(BF)
                    out_s[jj, r0:r0 + 16] = v
                    od.note(pltpu.bitcast(v, U32))
                yield 1

        def dx_proj(j, m, od):
            for k in range(7):
                m.append(od.dot(aq[k + z], _bf(gq[k + z, :, j * CG:(j + 1) * CG]), NN))
                yield 1

        def finish_dx(j, m, od):
            for r in range(0, HD, 16):
                q = _combine([v[r:r + 16] for v in m])
                for jj, r0, v in ((j, r, q[0]), (j + 2, r, q[1]), (j, HD + r, q[2]), (j + 2, HD + r, q[3])):
                    v = dxc[jj + z, r0:r0 + 16] + v
                    dxb[jj, r0:r0 + 16] = v
                    od.note_all(pltpu.bitcast(v, U32))
                yield 1

        def ln1_bwd(j, od):
            m1, r1 = ln_s[j, 0, 0:1], ln_s[j, 1, 0:1]

            def xn(r):
                return (_f(xT[j, r:r + 32]) - m1) * r1
            s1 = s2 = None
            for r in range(0, D, 32):
                d = dxb[j + z, r:r + 32]
                v1, v2 = _fold(d), _fold(d * xn(r))
                s1, s2 = (v1, v2) if r == 0 else (s1 + v1, s2 + v2)
                od.note(s1, s2)
                yield 1
            a1, a2 = _mean(s1), _mean(s2)
            for r in range(0, D, 32):
                v = (_f(gT[j, r:r + 32]) + r1 * (dxb[j + z, r:r + 32] - a1 - xn(r) * a2)).astype(BF)
                dx_s[j, r:r + 32] = v
                od.note_all(pltpu.bitcast(v, U32))
                yield 1

        def dwqkv_proj(c0, c1, n, od):
            for k in range(7):
                n.append(od.dot(tx[k], _bf(gq[k + z, c0 // 2:c1 // 2]), NT))
                yield 1

        def finish_dwqkv(c0, c1, n, od):
            c2 = min(c1, 3 * D - KQ)
            for r in range(0, HD, 16):
                q = _combine_t([v[r:r + 16] for v in n])
                for r0, u, l in ((r, q[0], q[1]), (HD + r, q[2], q[3])):
                    u, l = u.astype(BF), l.astype(BF)
                    dwqkv_s[r0:r0 + 16, c0:c1] = u
                    dwqkv_s[r0:r0 + 16, KQ + c0:KQ + c2] = l[:, 0:c2 - c0]
                    od.note(pltpu.bitcast(u, U32), pltpu.bitcast(l, U32))
                yield 1

        def dwo_proj(n, od):
            for k in range(7):
                n.append(od.dot(tg[1, k], _bf(go[k + z, 0:KS[k] // 2]), NT))
                yield 1

        def finish_dwo(n, od):
            q = _combine_t([v[:, 0:256] for v in n])
            ru = n[2][:, 256:] - n[5][:, 256:] + n[6][:, 256:]
            rl = n[3][:, 256:] + n[5][:, 256:] - n[6][:, 256:]
            t = _rows(_cols(q[0], q[1], ru), _cols(q[2], q[3], rl), jnp.zeros((64, 640), F32)).astype(BF).T
            dwo_s[...] = t[0:D, 0:D]
            db2_ref[...] = _f(t[D:D + 16, 0:D])[0:1].reshape(D).astype(BF)
            od.note_all(pltpu.bitcast(t, U32))
            yield 1

        dwqkv_out = [pltpu.make_async_copy(dwqkv_s.at[:, c0:c1], dwqkv_hbm.at[:, c0:c1], sem_dw.at[u])
                     for u, (c0, c1) in enumerate(((0, 640), (KQ, KQ + 640), (640, KQ), (KQ + 640, 3 * D)))]
        dwo_out = pltpu.make_async_copy(dwo_s, dwo_hbm, sem_dw.at[4])
        od = _Order(zero_s[0])
        n1, n2, mo0, mo1, no, mx0, mx1, nq0, nq1 = [], [], [], [], [], [], [], [], []
        att = _chain(*[attn_stage2(0, hg, od) for hg in range(4)])
        dq, of, l0, l1 = dq_forms(od), o_forms(od), ln2_bwd(0, od), ln2_bwd(1, od)
        _segment(od, stage_e(NCH - 1, 0, n1, od), 7, (att, 4 * N2), (wo_forms(od), 18), (_take(of, 15), 15), end=False)
        for q in range(2):
            d_cp(NCH - 2, q).wait()
        _segment(od, stage_e(NCH - 1, 1, n2, od), 7, (finish_e(0, n1, od), 6), (of, 25), (_take(dq, 14), 14))
        d_cp(NCH - 1, 0).start()
        _segment(od, out_proj(0, mo0, od), 7, (finish_e(1, n2, od), 6), (_take(dq, 11), 11), end=False)
        d_cp(NCH - 1, 1).start()
        _segment(od, out_proj(1, mo1, od), 7, (finish_out(0, mo0, od), 18), (_take(dq, 11), 11))
        o_cp(0).start()
        o_cp(2).start()
        _segment(od, dwo_proj(no, od), 7, (finish_out(1, mo1, od), 18), (dq, 20), (wq_forms(od), 18))
        o_cp(1).start()
        o_cp(3).start()
        _segment(od, dx_proj(0, mx0, od), 7, (finish_dwo(no, od), 1), (l0, 72))
        dwo_out.start()
        _segment(od, dx_proj(1, mx1, od), 7, (finish_dx(0, mx0, od), 18), (l1, 72))
        _segment(od, dwqkv_proj(0, 640, nq0, od), 7,
              (_chain(ln1_bwd(0, od), ln1_bwd(2, od), finish_dx(1, mx1, od), ln1_bwd(1, od)), 3 * 36 + 18))
        for j in (0, 2, 1):
            dx_cp(j).start()
        last = dwqkv_proj(640, KQ, nq1, od)
        _segment(od, _take(last, 2), 2, (finish_dwqkv(0, 640, nq0, od), 18))
        for cp in dwqkv_out[0:2]:
            cp.start()
        _segment(od, _take(last, 3), 3, (ln1_bwd(3, od), 36))
        dx_cp(3).start()
        _run(last)
        db1 = _cols(*[jnp.sum(db1s[i, 0] + db1s[i, 1], axis=0, keepdims=True) for i in range(NCH)])
        db1_ref[...] = db1.reshape(F).astype(BF)
        _run(finish_dwqkv(640, KQ, nq1, od))
        for cp in dwqkv_out[2:4]:
            cp.start()
        for q in range(2):
            d_cp(NCH - 1, q).wait()
        for j in range(NG):
            o_cp(j).wait()
            dx_cp(j).wait()
        for cp in dwqkv_out:
            cp.wait()
        dwo_out.wait()

    pl.run_scoped(epilogue, V((7, KQ // 2, HS), U32), V((7, 192, HS), U32), V((7, HD // 2, KQ), U32),
                  V((7, HD // 2, 384), U32), V((NG, D, CG), BF), V((NG, D, CG), BF), V((D, 3 * D), BF), V((D, D), BF),
                  V((NG, D, CG), F32), V((NG, D, CG), F32))


@jax.jit
def pallas_parallel_sum__sliding_local_dilated__mixer_channel_mlp__prompt_kernel(
    A_x, A_wqkv, A_wo, B_x, B_w1, B_b1, B_w2, B_b2, grad_out,
):
    del B_x
    hbm = pl.BlockSpec(memory_space=pl.ANY)
    vmem = pl.BlockSpec(memory_space=pltpu.VMEM)
    V = pltpu.VMEM
    dma = pltpu.SemaphoreType.DMA
    outs = pl.pallas_call(
        _kernel,
        in_specs=[hbm, hbm, hbm, hbm, hbm, vmem, hbm, vmem],
        out_specs=[hbm, hbm, hbm, hbm, hbm, vmem, hbm, vmem],
        out_shape=[
            jax.ShapeDtypeStruct((D, S), BF), jax.ShapeDtypeStruct((D, S), BF),
            jax.ShapeDtypeStruct((D, 3 * D), BF), jax.ShapeDtypeStruct((D, D), BF),
            jax.ShapeDtypeStruct((D, F), BF), jax.ShapeDtypeStruct((F,), BF),
            jax.ShapeDtypeStruct((D, F), BF), jax.ShapeDtypeStruct((D,), BF),
        ],
        scratch_shapes=[
            V((NG, D, CG), BF), V((NG, D, CG), BF), V((D, 3 * D), BF), V((D, D), BF),
            V((2, 7, HD // 2, HS), U32), V((7, HD // 2, HS), U32),
            V((NB, DP, 128), U32), V((NB, 3 * DP, 128), U32), V((2, 2, 7, HD, CG), F32),
            V((2, 2, 2, 7, CG // 2, HF), U32), V((NB + 1, DP, 128), U32), V((NB + 1, DP, 128), U32),
            V((4, W, H, 128), F32), V((4, W, H, 128), F32), V((NCH, 2, 8, FC), F32),
            V((NG, 4, 8, CG), F32),             V((2, 8, 128), U32), V((2, D, FC), BF),
            dma((NG,)), dma((NG,)), dma((5,)), dma((4,)), dma((2,)), dma((NG,)), dma((NG,)), dma((5,)),
        ],
        compiler_params=pltpu.CompilerParams(vmem_limit_bytes=128 * 2**20),
    )(A_x[0].T, grad_out[0].T, A_wqkv, A_wo, B_w1, B_b1, B_w2.T, B_b2)
    outT, dxT, dwqkv, dwo, dw1, db1, dw2T, db2 = outs
    return (outT.T[None], dxT.T[None], dwqkv, dwo, dw1, db1, dw2T.T, db2)
```
